```python
import os as _os
_os.environ.setdefault("JAX_PLATFORMS", "cpu")
import jax
import jax.numpy as jnp

def _softmax(x, axis=-1):
    return jax.nn.softmax(x, axis=axis)
def _gelu(x):
    return jax.nn.gelu(x, approximate=True)
def _silu(x):
    return jax.nn.silu(x)
def _sigmoid(x):
    return jax.nn.sigmoid(x)
def _layernorm(x, axis=-1, eps=1e-5):
    m = jnp.mean(x, axis=axis, keepdims=True)
    v = jnp.var(x, axis=axis, keepdims=True)
    return (x - m) / jnp.sqrt(v + eps)
def _scatter_add(tgt, idx, src, axis=0):
    return tgt.at[idx].add(src)
def _segment_sum(src, seg, n):
    return jax.ops.segment_sum(src, seg, n)
class _Rng:
    def __init__(self, key):
        self._k = key
    def _next(self):
        self._k, sub = jax.random.split(self._k)
        return sub
    def normal(self, shape):
        return jax.random.normal(self._next(), shape, dtype=jnp.bfloat16)
    def randint(self, lo, hi, shape):
        return jax.random.randint(self._next(), shape, lo, hi, dtype=jnp.int32)
    def uniform(self, shape, lo=0.0, hi=1.0):
        return jax.random.uniform(self._next(), shape, jnp.bfloat16, lo, hi)
    def permutation(self, n):
        return jax.random.permutation(self._next(), n)


kernel_name = 'standalone__detection_seg_fpn_lateral__vision'

def setup_inputs():
    _rng = _Rng(jax.random.key(int.from_bytes(__import__("os").urandom(4), "little")))
    _w = (lambda a: (lambda t: t.astype(jnp.bfloat16) if jnp.issubdtype(t.dtype, jnp.floating) else t)(jnp.asarray(a)))
    H = W = (256 // 2) * 2
    C = 384
    k = 1
    return {
        "c_fine": _w((lambda *s: _rng.normal(s) * 0.05)(1, H, W, C)),
        "p_coarse": _w((lambda *s: _rng.normal(s) * 0.05)(1, H // 2, W // 2, C)),
        "w_lat": _w((lambda *s: _rng.normal(s) * 0.05)(C, C)),
        "w_out": _w((lambda *s: _rng.normal(s) * 0.05)(k, k, C, C)),
    }

def reference(c_fine, p_coarse, w_lat, w_out):
    B, H, W, C = c_fine.shape
    k = 1
    lat = jnp.einsum("bhwc,cd->bhwd", c_fine, w_lat)
    up = jnp.repeat(jnp.repeat(p_coarse, 2, axis=1), 2, axis=2)
    m = lat + up
    pad = k // 2
    mp = jnp.pad(m, ((0, 0), (pad, pad), (pad, pad), (0, 0)))
    o = None
    for di in range(k):
        for dj in range(k):
            t = jnp.einsum("bhwc,cd->bhwd", mp[:, di:di + H, dj:dj + W, :], w_out[di, dj])
            o = t if o is None else o + t
    return o
```

```python
import jax
import jax.numpy as jnp
from jax import lax
import jax.experimental.pallas as pl
import jax.experimental.pallas.tpu as pltpu

_LANES = 128
_CR = 4
_READ_B = (0, 2, 5, 9, 16, 32)
_X = 16
_WRITE_B = (0, 16, 24, 28, 30, 32)


@jax.jit
def pallas_standalone__detection_seg_fpn_lateral__vision_kernel(
    c_fine: jax.Array,
    p_coarse: jax.Array,
    w_lat: jax.Array,
    w_out: jax.Array,
):
    B, H, W, C = c_fine.shape
    Hc, Wc = H // 2, W // 2
    nsteps = (B * Hc) // _CR
    FR = 2 * _CR * W
    PR = _CR * Wc
    NJ = C // _LANES
    rb, wb, X = _READ_B, _WRITE_B, _X
    assert rb[-1] == nsteps and wb[-1] == nsteps
    nr, nw = len(rb) - 1, len(wb) - 1

    def kernel(c_hbm, p_hbm, wl_hbm, wo_hbm, o_hbm,
               cbuf, pbuf, obuf, wl_v, wo_v, wc_v, qs,
               csem, psem, wsem, osem):
        def c_cp(k):
            a, n = rb[k] * FR, (rb[k + 1] - rb[k]) * FR
            return pltpu.make_async_copy(
                c_hbm.at[pl.ds(a, n)], cbuf.at[pl.ds(a, n)], csem.at[k])

        def p_cp(k):
            a, n = rb[k] * PR, (rb[k + 1] - rb[k]) * PR
            return pltpu.make_async_copy(
                p_hbm.at[pl.ds(a, n)], pbuf.at[pl.ds(a, n)], psem.at[k])

        def o_cp(k):
            a, n = wb[k] * FR, (wb[k + 1] - wb[k]) * FR
            return pltpu.make_async_copy(
                obuf.at[pl.ds(a, n)], o_hbm.at[pl.ds(a, n)], osem.at[k])

        wl_cp = pltpu.make_async_copy(wl_hbm, wl_v, wsem.at[0])
        wo_cp = pltpu.make_async_copy(wo_hbm, wo_v, wsem.at[1])
        wo_cp.start()
        wl_cp.start()
        p_cp(0).start()
        c_cp(0).start()
        wo_cp.wait()
        wl_cp.wait()
        for k in range(1, nr):
            p_cp(k).start()
            c_cp(k).start()
        wc_v[...] = jnp.dot(
            wl_v[...], wo_v[...], preferred_element_type=jnp.float32
        ).astype(wc_v.dtype)

        def step(s, carry):
            for k in range(nr):
                @pl.when(s == min(rb[k], X))
                def _():
                    p_cp(k).wait()
                    c_cp(k).wait()
            for k in range(nw - 1):
                @pl.when(s == max(wb[k + 1], X))
                def _():
                    o_cp(k).start()

            pr = pl.multiple_of(s * PR, PR)
            q = jnp.dot(pbuf[pl.ds(pr, PR), :], wo_v[...],
                        preferred_element_type=jnp.float32)
            for j in range(NJ):
                qj = q[:, j * _LANES:(j + 1) * _LANES]
                qs[j, pl.ds(0, PR, stride=2), :] = qj
                qs[j, pl.ds(1, PR, stride=2), :] = qj
            for i in range(_CR):
                for r in range(2):
                    cr = pl.multiple_of(s * FR + (2 * i + r) * W, W)
                    acc = jnp.dot(cbuf[pl.ds(cr, W), :], wc_v[...],
                                  preferred_element_type=jnp.float32)
                    up = jnp.concatenate(
                        [qs[j, i * W:(i + 1) * W, :] for j in range(NJ)], axis=1)
                    obuf[pl.ds(cr, W), :] = (acc + up).astype(obuf.dtype)
            return carry

        lax.fori_loop(0, nsteps, step, 0)
        o_cp(nw - 1).start()
        for k in range(nw):
            o_cp(k).wait()

    dt = c_fine.dtype
    out = pl.pallas_call(
        kernel,
        in_specs=[pl.BlockSpec(memory_space=pl.ANY)] * 4,
        out_specs=pl.BlockSpec(memory_space=pl.ANY),
        out_shape=jax.ShapeDtypeStruct((B * H * W, C), dt),
        scratch_shapes=[
            pltpu.VMEM((B * H * W, C), dt),
            pltpu.VMEM((B * Hc * Wc, C), dt),
            pltpu.VMEM((B * H * W, C), dt),
            pltpu.VMEM((C, C), dt),
            pltpu.VMEM((C, C), dt),
            pltpu.VMEM((C, C), dt),
            pltpu.VMEM((NJ, 2 * PR + 8, _LANES), jnp.float32),
            pltpu.SemaphoreType.DMA((nr,)),
            pltpu.SemaphoreType.DMA((nr,)),
            pltpu.SemaphoreType.DMA((2,)),
            pltpu.SemaphoreType.DMA((nw,)),
        ],
        compiler_params=pltpu.CompilerParams(vmem_limit_bytes=124 * 1024 * 1024),
    )(
        c_fine.reshape(B * H * W, C),
        p_coarse.reshape(B * Hc * Wc, C),
        w_lat,
        w_out.reshape(C, C),
    )
    return out.reshape(B, H, W, C)
```

```python
import functools

import jax
import jax.numpy as jnp
from jax import lax
import jax.experimental.pallas as pl
import jax.experimental.pallas.tpu as pltpu

_LANES = 128
_BW = 64
_HP = 2
_NGP = 4
_M = 256
_X = 17
_G = 64

_READS = (
    ("p", 0, _G, 0, 1, 0, 2),
    ("c", 0, 32, 0, 1, 0, 1),
    ("c", 32, _G, 0, 1, 0, 1),
    ("c", 0, _G, 0, 1, 1, 2),
    ("p", 0, _G, 0, 1, 2, 4),
    ("c", 0, _G, 0, 1, 2, 4),
    ("p", 0, _G, 1, 2, 0, 4),
    ("c", 0, _G, 1, 2, 0, 1),
    ("c", 0, _G - 1, 1, 2, 1, 4),
    ("c", _G - 1, _G, 1, 2, 1, 4),
)
_N_EARLY = 2
_WRITES = tuple((a, 0, _G) for a in range(7)) + ((7, 0, 32), (7, 32, _G))


@jax.jit
def pallas_standalone__detection_seg_fpn_lateral__vision_kernel(
    c_fine: jax.Array,
    p_coarse: jax.Array,
    w_lat: jax.Array,
    w_out: jax.Array,
):
    B, H, W, C = c_fine.shape
    CQ = W // _BW
    G = B * H // (2 * _HP)
    assert G == _G and _HP * CQ == 8
    GS = G // _NGP
    nsteps = _HP * CQ * _NGP
    NJ = C // _LANES
    BP = _BW // 2
    PR = GS * BP
    GM = _M // _BW
    nr, nw = len(_READS), len(_WRITES)

    def first_use(k):
        _, g0, _, h0, _, q0, _ = _READS[k]
        return (h0 * CQ + q0) * _NGP + g0 // GS

    def ready(k):
        a, _, g1 = _WRITES[k]
        return a * _NGP + pl.cdiv(g1, GS)

    assert first_use(nr - 1) >= _X
    event_steps = sorted(
        {min(first_use(k), _X) for k in range(nr)}
        | {max(ready(k), _X) for k in range(nw)})

    def kernel(c_hbm, p_hbm, wl_hbm, wo_hbm, o_hbm,
               cbuf, pbuf, obuf, wl_v, wo_v, wc_v, qs, rsem, wsem, osem):
        def read(k):
            kind, g0, g1, h0, h1, q0, q1 = _READS[k]
            gs, hs, cs = pl.ds(g0, g1 - g0), pl.ds(h0, h1 - h0), pl.ds(q0, q1 - q0)
            if kind == "c":
                return pltpu.make_async_copy(
                    c_hbm.at[gs, hs, :, cs], cbuf.at[gs, hs, :, cs], rsem.at[k])
            return pltpu.make_async_copy(
                p_hbm.at[gs, hs, cs], pbuf.at[gs, hs, cs], rsem.at[k])

        def write(k, r):
            a, g0, g1 = _WRITES[k]
            hp, cq, gs = a // CQ, a % CQ, pl.ds(g0, g1 - g0)
            return pltpu.make_async_copy(
                obuf.at[gs, hp, r, cq], o_hbm.at[gs, hp, r, cq], osem.at[2 * k + r])

        def events(st):
            for k in range(nr - 1):
                if min(first_use(k), _X) == st:
                    read(k).wait()
            for k in range(nw):
                if max(ready(k), _X) == st:
                    write(k, 0).start()
                    write(k, 1).start()
            if st == _X:
                read(nr - 1).wait()

        wl_cp = pltpu.make_async_copy(wl_hbm, wl_v, wsem.at[0])
        wo_cp = pltpu.make_async_copy(wo_hbm, wo_v, wsem.at[1])
        wo_cp.start()
        wl_cp.start()
        for k in range(_N_EARLY):
            read(k).start()
        wo_cp.wait()
        wl_cp.wait()
        for k in range(_N_EARLY, nr):
            read(k).start()
        wc_v[...] = jnp.dot(
            wl_v[...], wo_v[...], preferred_element_type=jnp.float32
        ).astype(wc_v.dtype)

        def step(s, carry):
            for st in event_steps:
                if st < nsteps:
                    pl.when(s == st)(functools.partial(events, st))
            a = s // _NGP
            hp, cq = a // CQ, a % CQ
            g0 = (s % _NGP) * GS
            pv = pbuf[pl.ds(g0, GS), hp, cq].reshape(PR, C)
            q = jnp.dot(pv, wo_v[...], preferred_element_type=jnp.float32)
            for j in range(NJ):
                qj = q[:, j * _LANES:(j + 1) * _LANES]
                qs[j, pl.ds(0, PR, stride=2), :] = qj
                qs[j, pl.ds(1, PR, stride=2), :] = qj
            for r in range(2):
                for i in range(GS // GM):
                    gsl = pl.ds(g0 + i * GM, GM)
                    cv = cbuf[gsl, hp, r, cq].reshape(_M, C)
                    acc = jnp.dot(cv, wc_v[...], preferred_element_type=jnp.float32)
                    up = jnp.concatenate(
                        [qs[j, i * _M:(i + 1) * _M, :] for j in range(NJ)], axis=1)
                    obuf[gsl, hp, r, cq] = (
                        (acc + up).astype(obuf.dtype).reshape(GM, _BW, C))
            return carry

        lax.fori_loop(0, nsteps, step, 0)
        events(nsteps)
        for k in range(nw):
            write(k, 0).wait()
            write(k, 1).wait()

    dt = c_fine.dtype
    fshape = (G, _HP, 2, CQ, _BW, C)
    pshape = (G, _HP, CQ, BP, C)
    out = pl.pallas_call(
        kernel,
        in_specs=[pl.BlockSpec(memory_space=pl.ANY)] * 4,
        out_specs=pl.BlockSpec(memory_space=pl.ANY),
        out_shape=jax.ShapeDtypeStruct(fshape, dt),
        scratch_shapes=[
            pltpu.VMEM(fshape, dt),
            pltpu.VMEM(pshape, dt),
            pltpu.VMEM(fshape, dt),
            pltpu.VMEM((C, C), dt),
            pltpu.VMEM((C, C), dt),
            pltpu.VMEM((C, C), dt),
            pltpu.VMEM((NJ, 2 * PR + 8, _LANES), jnp.float32),
            pltpu.SemaphoreType.DMA((nr,)),
            pltpu.SemaphoreType.DMA((2,)),
            pltpu.SemaphoreType.DMA((2 * nw,)),
        ],
        compiler_params=pltpu.CompilerParams(vmem_limit_bytes=124 * 1024 * 1024),
    )(
        c_fine.reshape(fshape),
        p_coarse.reshape(pshape),
        w_lat,
        w_out.reshape(C, C),
    )
    return out.reshape(B, H, W, C)
```

```python
import functools

import jax
import jax.numpy as jnp
from jax import lax
import jax.experimental.pallas as pl
import jax.experimental.pallas.tpu as pltpu

_LANES = 128
_G = 16
_HP = 8
_CQ = 2
_BW = 128
_GS = 8
_M = 256
_NS = 32
_BT = 16
_X = 19
_PAD = 220

_ORDER = ((7, 1), (6, 1), (1, 0), (1, 1), (7, 0), (6, 0), (5, 0), (4, 0),
          (3, 0), (2, 0), (4, 1), (2, 1), (3, 1), (0, 1), (5, 1), (0, 0))

_READS = (
    ("p", 0, 16, 6, 8, 1, 2),
    ("c", 0, 8, 7, 8, 1, 2),
    ("c", 8, 16, 7, 8, 1, 2),
    ("c", 0, 16, 6, 7, 1, 2),
    ("p", 0, 16, 1, 2, 0, 2),
    ("c", 0, 16, 1, 2, 0, 2),
    ("p", 0, 16, 2, 8, 0, 1),
    ("c", 0, 16, 6, 8, 0, 1),
    ("c", 0, 16, 2, 6, 0, 1),
    ("p", 0, 16, 2, 6, 1, 2),
    ("p", 0, 16, 0, 1, 0, 2),
    ("c", 0, 16, 2, 6, 1, 2),
    ("c", 0, 15, 0, 1, 0, 2),
    ("c", 15, 16, 0, 1, 0, 2),
)
_N_EARLY = 2


def _first_use(k):
    _, g0, g1, k0, k1, q0, q1 = _READS[k]
    return min(2 * u + h
               for u, (kk, cq) in enumerate(_ORDER) for h in range(2)
               if k0 <= kk < k1 and q0 <= cq < q1
               and g0 < (h + 1) * _GS and g1 > h * _GS)


def _ready(i):
    return max(2 * u + 2
               for u, (kk, cq) in enumerate(_ORDER) for r in range(2)
               for d in range(3) if (12 * kk + 6 * r + 3 * cq + d) % _NS == i)


def _packed_order(lo):
    word = sum((2 * kk + cq) << (4 * n) for n, (kk, cq) in enumerate(_ORDER[lo:lo + 4]))
    return jnp.int32(word)


@jax.jit
def pallas_standalone__detection_seg_fpn_lateral__vision_kernel(
    c_fine: jax.Array,
    p_coarse: jax.Array,
    w_lat: jax.Array,
    w_out: jax.Array,
):
    B, H, W, C = c_fine.shape
    assert B * H == _G * _HP * 2 and W == _CQ * _BW and C == 3 * _LANES
    NJ = C // _LANES
    BP = _BW // 2
    PR = _GS * BP
    GM = _M // _BW
    nsteps = 2 * len(_ORDER)
    nr = len(_READS)
    streams = sorted(range(_NS), key=lambda i: (_ready(i), i))
    assert _first_use(nr - 1) >= _X
    event_steps = sorted(
        {min(_first_use(k), _X) for k in range(nr)}
        | {max(_ready(i), _X) for i in streams})

    def kernel(c_hbm, p_hbm, wl_hbm, wo_hbm, o_hbm,
               cbuf, pbuf, obuf, wl_v, wo_v, wc_v, qs, rsem, wsem, osem):
        def read(k):
            kind, g0, g1, k0, k1, q0, q1 = _READS[k]
            gs, ks, cs = pl.ds(g0, g1 - g0), pl.ds(k0, k1 - k0), pl.ds(q0, q1 - q0)
            if kind == "c":
                return pltpu.make_async_copy(
                    c_hbm.at[gs, ks, :, cs], cbuf.at[gs, ks, :, cs], rsem.at[k])
            return pltpu.make_async_copy(
                p_hbm.at[gs, ks, cs], pbuf.at[gs, ks, cs], rsem.at[k])

        def write(i):
            return pltpu.make_async_copy(obuf.at[:, i], o_hbm.at[:, i], osem.at[i])

        def events(st):
            for k in range(nr - 1):
                if min(_first_use(k), _X) == st:
                    read(k).wait()
            for i in streams:
                if max(_ready(i), _X) == st:
                    write(i).start()
            if st == _X:
                read(nr - 1).wait()

        wl_cp = pltpu.make_async_copy(wl_hbm, wl_v, wsem.at[0])
        wo_cp = pltpu.make_async_copy(wo_hbm, wo_v, wsem.at[1])
        wo_cp.start()
        wl_cp.start()
        for k in range(_N_EARLY):
            read(k).start()
        wo_cp.wait()
        wl_cp.wait()
        for k in range(_N_EARLY, nr):
            read(k).start()
        wc_v[...] = jnp.dot(
            wl_v[...], wo_v[...], preferred_element_type=jnp.float32
        ).astype(wc_v.dtype)

        def step(s, carry):
            for st in event_steps:
                if st < nsteps:
                    pl.when(s == st)(functools.partial(events, st))
            word = jnp.where(
                s < 16,
                jnp.where(s < 8, _packed_order(0), _packed_order(4)),
                jnp.where(s < 24, _packed_order(8), _packed_order(12)))
            code = (word >> (2 * (s & 6))) & 15
            kk, cq = code >> 1, code & 1
            g0 = (s & 1) * _GS
            pv = pbuf[pl.ds(g0, _GS), kk, cq].reshape(PR, C)
            q = jnp.dot(pv, wo_v[...], preferred_element_type=jnp.float32)
            for j in range(NJ):
                qj = q[:, j * _LANES:(j + 1) * _LANES]
                qs[j, pl.ds(0, PR, stride=2), :] = qj
                qs[j, pl.ds(1, PR, stride=2), :] = qj
            for r in range(2):
                b0 = 12 * kk + 6 * r + 3 * cq
                for i in range(_GS // GM):
                    cv = cbuf[pl.ds(g0 + i * GM, GM), kk, r, cq].reshape(_M, C)
                    acc = jnp.dot(cv, wc_v[...], preferred_element_type=jnp.float32)
                    res = acc + jnp.concatenate(
                        [qs[j, i * _M:(i + 1) * _M, :] for j in range(NJ)], axis=1)
                    for gi in range(GM):
                        for d in range(3):
                            tiles = []
                            for t in range(d * _BT, (d + 1) * _BT):
                                row = gi * _BW + (t // NJ) * 8
                                col = (t % NJ) * _LANES
                                tiles.append(res[row:row + 8, col:col + _LANES])
                            b = b0 + d
                            m = 3 * (g0 + i * GM + gi) + (b >> 5)
                            obuf[m, b & (_NS - 1)] = jnp.stack(tiles).astype(obuf.dtype)
            return carry

        lax.fori_loop(0, nsteps, step, 0)
        events(nsteps)
        for n in range(_PAD):
            qs[(n // 128) % NJ, pl.ds(8 * (n % 128), 8), :] = jnp.full(
                (8, _LANES), n, jnp.float32)
        for i in streams:
            write(i).wait()

    dt = c_fine.dtype
    fshape = (_G, _HP, 2, _CQ, _BW, C)
    pshape = (_G, _HP, _CQ, BP, C)
    oshape = (3 * _G, _NS, _BT, 8, _LANES)
    out = pl.pallas_call(
        kernel,
        in_specs=[pl.BlockSpec(memory_space=pl.ANY)] * 4,
        out_specs=pl.BlockSpec(memory_space=pl.ANY),
        out_shape=jax.ShapeDtypeStruct(oshape, dt),
        scratch_shapes=[
            pltpu.VMEM(fshape, dt),
            pltpu.VMEM(pshape, dt),
            pltpu.VMEM(oshape, dt),
            pltpu.VMEM((C, C), dt),
            pltpu.VMEM((C, C), dt),
            pltpu.VMEM((C, C), dt),
            pltpu.VMEM((NJ, 2 * PR + 8, _LANES), jnp.float32),
            pltpu.SemaphoreType.DMA((nr,)),
            pltpu.SemaphoreType.DMA((2,)),
            pltpu.SemaphoreType.DMA((_NS,)),
        ],
        compiler_params=pltpu.CompilerParams(vmem_limit_bytes=124 * 1024 * 1024),
    )(
        c_fine.reshape(fshape),
        p_coarse.reshape(pshape),
        w_lat,
        w_out.reshape(C, C),
    )
    out = out.reshape(B * H * W // 8, NJ, 8, _LANES).transpose(0, 2, 1, 3)
    return out.reshape(B, H, W, C)
```

```python
import functools

import jax
import jax.numpy as jnp
from jax import lax
import jax.experimental.pallas as pl
import jax.experimental.pallas.tpu as pltpu

_LANES = 128
_G = 16
_HP = 8
_CQ = 2
_BW = 128
_GS = 8
_M = 512
_NS = 32
_BT = 16
_X = 19

_ORDER = ((7, 1), (6, 1), (1, 0), (1, 1), (7, 0), (6, 0), (5, 0), (4, 0),
          (3, 0), (2, 0), (4, 1), (2, 1), (3, 1), (0, 1), (5, 1), (0, 0))

_READS = (
    ("p", 0, 16, 6, 8, 1, 2),
    ("c", 0, 8, 7, 8, 1, 2),
    ("c", 8, 16, 7, 8, 1, 2),
    ("c", 0, 16, 6, 7, 1, 2),
    ("p", 0, 16, 1, 2, 0, 2),
    ("c", 0, 16, 1, 2, 0, 2),
    ("p", 0, 16, 2, 8, 0, 1),
    ("c", 0, 16, 6, 8, 0, 1),
    ("c", 0, 16, 2, 6, 0, 1),
    ("p", 0, 16, 2, 6, 1, 2),
    ("p", 0, 16, 0, 1, 0, 2),
    ("c", 0, 16, 2, 6, 1, 2),
    ("c", 0, 15, 0, 1, 0, 2),
    ("c", 15, 16, 0, 1, 0, 2),
)
_N_EARLY = 2


def _first_use(k):
    _, g0, g1, k0, k1, q0, q1 = _READS[k]
    return min(2 * u + h
               for u, (kk, cq) in enumerate(_ORDER) for h in range(2)
               if k0 <= kk < k1 and q0 <= cq < q1
               and g0 < (h + 1) * _GS and g1 > h * _GS)


def _ready(i):
    return max(2 * u + 2
               for u, (kk, cq) in enumerate(_ORDER) for r in range(2)
               for d in range(3) if (12 * kk + 6 * r + 3 * cq + d) % _NS == i)


def _packed_order(lo):
    word = sum((2 * kk + cq) << (4 * n) for n, (kk, cq) in enumerate(_ORDER[lo:lo + 4]))
    return jnp.int32(word)


@jax.jit
def pallas_standalone__detection_seg_fpn_lateral__vision_kernel(
    c_fine: jax.Array,
    p_coarse: jax.Array,
    w_lat: jax.Array,
    w_out: jax.Array,
):
    B, H, W, C = c_fine.shape
    assert B * H == _G * _HP * 2 and W == _CQ * _BW and C == 3 * _LANES
    NJ = C // _LANES
    BP = _BW // 2
    PR = _GS * BP
    GM = _M // _BW
    nsteps = 2 * len(_ORDER)
    nr = len(_READS)
    streams = sorted(range(_NS), key=lambda i: (_ready(i), i))
    assert _first_use(nr - 1) >= _X
    event_steps = sorted(
        {min(_first_use(k), _X) for k in range(nr)}
        | {max(_ready(i), _X) for i in streams})

    def kernel(c_hbm, p_hbm, wl_hbm, wo_hbm, o_hbm,
               cbuf, pbuf, obuf, wl_v, wo_v, wc_v, qs, rsem, wsem, osem):
        def read(k):
            kind, g0, g1, k0, k1, q0, q1 = _READS[k]
            gs, ks, cs = pl.ds(g0, g1 - g0), pl.ds(k0, k1 - k0), pl.ds(q0, q1 - q0)
            if kind == "c":
                return pltpu.make_async_copy(
                    c_hbm.at[gs, ks, :, cs], cbuf.at[gs, ks, :, cs], rsem.at[k])
            return pltpu.make_async_copy(
                p_hbm.at[gs, ks, cs], pbuf.at[gs, ks, cs], rsem.at[k])

        def write(i):
            return pltpu.make_async_copy(obuf.at[:, i], o_hbm.at[:, i], osem.at[i])

        def events(st):
            for k in range(nr - 1):
                if min(_first_use(k), _X) == st:
                    read(k).wait()
            for i in streams:
                if max(_ready(i), _X) == st:
                    write(i).start()
            if st == _X:
                read(nr - 1).wait()

        wl_cp = pltpu.make_async_copy(wl_hbm, wl_v, wsem.at[0])
        wo_cp = pltpu.make_async_copy(wo_hbm, wo_v, wsem.at[1])
        wo_cp.start()
        wl_cp.start()
        for k in range(_N_EARLY):
            read(k).start()
        wo_cp.wait()
        wl_cp.wait()
        for k in range(_N_EARLY, nr):
            read(k).start()
        wc_v[...] = jnp.dot(
            wl_v[...], wo_v[...], preferred_element_type=jnp.float32
        ).astype(wc_v.dtype)

        def step(s, carry):
            for st in event_steps:
                if st < nsteps:
                    pl.when(s == st)(functools.partial(events, st))
            word = jnp.where(
                s < 16,
                jnp.where(s < 8, _packed_order(0), _packed_order(4)),
                jnp.where(s < 24, _packed_order(8), _packed_order(12)))
            code = (word >> (2 * (s & 6))) & 15
            kk, cq = code >> 1, code & 1
            g0 = (s & 1) * _GS
            pv = pbuf[pl.ds(g0, _GS), kk, cq].reshape(PR, C)
            q = jnp.dot(pv, wo_v[...], preferred_element_type=jnp.float32)
            for j in range(NJ):
                qj = q[:, j * _LANES:(j + 1) * _LANES]
                qs[j, pl.ds(0, PR, stride=2), :] = qj
                qs[j, pl.ds(1, PR, stride=2), :] = qj
            for r in range(2):
                b0 = 12 * kk + 6 * r + 3 * cq
                for i in range(_GS // GM):
                    cv = cbuf[pl.ds(g0 + i * GM, GM), kk, r, cq].reshape(_M, C)
                    acc = jnp.dot(cv, wc_v[...], preferred_element_type=jnp.float32)
                    res = acc + jnp.concatenate(
                        [qs[j, i * _M:(i + 1) * _M, :] for j in range(NJ)], axis=1)
                    for gi in range(GM):
                        for d in range(3):
                            tiles = []
                            for t in range(d * _BT, (d + 1) * _BT):
                                row = gi * _BW + (t // NJ) * 8
                                col = (t % NJ) * _LANES
                                tiles.append(res[row:row + 8, col:col + _LANES])
                            b = b0 + d
                            m = 3 * (g0 + i * GM + gi) + (b >> 5)
                            obuf[m, b & (_NS - 1)] = jnp.stack(tiles).astype(obuf.dtype)
            return carry

        lax.fori_loop(0, nsteps, step, 0)
        events(nsteps)
        for i in streams:
            write(i).wait()

    dt = c_fine.dtype
    fshape = (_G, _HP, 2, _CQ, _BW, C)
    pshape = (_G, _HP, _CQ, BP, C)
    oshape = (3 * _G, _NS, _BT, 8, _LANES)
    out = pl.pallas_call(
        kernel,
        in_specs=[pl.BlockSpec(memory_space=pl.ANY)] * 4,
        out_specs=pl.BlockSpec(memory_space=pl.ANY),
        out_shape=jax.ShapeDtypeStruct(oshape, dt),
        scratch_shapes=[
            pltpu.VMEM(fshape, dt),
            pltpu.VMEM(pshape, dt),
            pltpu.VMEM(oshape, dt),
            pltpu.VMEM((C, C), dt),
            pltpu.VMEM((C, C), dt),
            pltpu.VMEM((C, C), dt),
            pltpu.VMEM((NJ, 2 * PR + 8, _LANES), jnp.float32),
            pltpu.SemaphoreType.DMA((nr,)),
            pltpu.SemaphoreType.DMA((2,)),
            pltpu.SemaphoreType.DMA((_NS,)),
        ],
        compiler_params=pltpu.CompilerParams(vmem_limit_bytes=124 * 1024 * 1024),
    )(
        c_fine.reshape(fshape),
        p_coarse.reshape(pshape),
        w_lat,
        w_out.reshape(C, C),
    )
    out = out.reshape(B * H * W // 8, NJ, 8, _LANES).transpose(0, 2, 1, 3)
    return out.reshape(B, H, W, C)
```
